```python
import os as _os
_os.environ.setdefault("JAX_PLATFORMS", "cpu")
import jax
import jax.numpy as jnp

def _softmax(x, axis=-1):
    return jax.nn.softmax(x, axis=axis)
def _gelu(x):
    return jax.nn.gelu(x, approximate=True)
def _silu(x):
    return jax.nn.silu(x)
def _sigmoid(x):
    return jax.nn.sigmoid(x)
def _layernorm(x, axis=-1, eps=1e-5):
    m = jnp.mean(x, axis=axis, keepdims=True)
    v = jnp.var(x, axis=axis, keepdims=True)
    return (x - m) / jnp.sqrt(v + eps)
def _scatter_add(tgt, idx, src, axis=0):
    return tgt.at[idx].add(src)
def _segment_sum(src, seg, n):
    return jax.ops.segment_sum(src, seg, n)
class _Rng:
    def __init__(self, key):
        self._k = key
    def _next(self):
        self._k, sub = jax.random.split(self._k)
        return sub
    def normal(self, shape):
        return jax.random.normal(self._next(), shape, dtype=jnp.bfloat16)
    def randint(self, lo, hi, shape):
        return jax.random.randint(self._next(), shape, lo, hi, dtype=jnp.int32)
    def uniform(self, shape, lo=0.0, hi=1.0):
        return jax.random.uniform(self._next(), shape, jnp.bfloat16, lo, hi)
    def permutation(self, n):
        return jax.random.permutation(self._next(), n)


kernel_name = 'interleave_layers__gqa_block_cached__dense_activation_mish__decode'

def setup_inputs():
    _rng = _Rng(jax.random.key(int.from_bytes(__import__("os").urandom(4), "little")))
    _w = (lambda a: (lambda t: t.astype(jnp.bfloat16) if jnp.issubdtype(t.dtype, jnp.floating) else t)(jnp.asarray(a)))
    def _A_setup():
        B, Sq, D = 1, 1, 512
        Hq, Hkv, Sk, Dh = 32, 8, 65536, 128
        assert Hq % Hkv == 0, (Hq, Hkv)
        return {
            "x": _w((lambda *s: _rng.normal(s) * 0.05)(B, Sq, D)),
            "k_cache": _w((lambda *s: _rng.normal(s) * 1.6)(B, Hkv, Sk, Dh)),
            "v_cache": _w((lambda *s: _rng.normal(s) * 1.6)(B, Hkv, Sk, Dh)),
            "wq": _w((lambda *s: _rng.normal(s) * 1.6)(D, Hq * Dh) * (D ** -0.5)),
            "wo": _w((lambda *s: _rng.normal(s) * 1.6)(Hq * Dh, D) * ((Hq * Dh) ** -0.5)),
        }
    _A_in = _A_setup()

    def _B_setup():
        B, S, D, F = 1, 1, 512, 1792
        return {
            "x": _w((lambda *s: _rng.normal(s) * 0.05)(B, S, D)),
            "w1": _w((lambda *s: _rng.normal(s) * 0.8)(D, F) * (D ** -0.5)),
            "b1": _w((lambda *s: _rng.normal(s) * 0.8)(F)),
            "w2": _w((lambda *s: _rng.normal(s) * 0.8)(F, D) * (F ** -0.5)),
        }
    _B_in = _B_setup()

    return {
        "A_x": _A_in["x"],
        "A_k_cache": _A_in["k_cache"],
        "A_v_cache": _A_in["v_cache"],
        "A_wq": _A_in["wq"],
        "A_wo": _A_in["wo"],
        "B_x": _B_in["x"],
        "B_w1": _B_in["w1"],
        "B_b1": _B_in["b1"],
        "B_w2": _B_in["w2"],
    }

def reference(A_x, A_k_cache, A_v_cache, A_wq, A_wo, B_x, B_w1, B_b1, B_w2):
    def _A_ref(x, k_cache, v_cache, wq, wo):
        B, Sq, D = x.shape
        Hq, Dh = 32, 128
        Hkv = k_cache.shape[1]
        rep = Hq // Hkv
        q = (lambda x, *d: x.transpose(*d))((x @ wq).reshape(B, Sq, Hq, Dh), 0, 2, 1, 3)
        k = jnp.repeat(k_cache, rep, axis=1)
        v = jnp.repeat(v_cache, rep, axis=1)
        scores = jnp.einsum("bhqd,bhkd->bhqk", q, k) * (Dh ** -0.5)
        p = _softmax(scores, axis=-1)
        o = jnp.einsum("bhqk,bhkd->bhqd", p, v)
        return (lambda x, *d: x.transpose(*d))(o, 0, 2, 1, 3).reshape(B, Sq, Hq * Dh) @ wo

    def _B_ref(x, w1, b1, w2):
        h = jnp.einsum("bsd,df->bsf", x, w1) + b1
        sp = jnp.log1p(jnp.exp(-jnp.abs(h))) + jnp.where(h > 0, h, jnp.zeros_like(h))
        act = h * jnp.tanh(sp)
        return jnp.einsum("bsf,fd->bsd", act, w2)

    x = A_x
    x = x + _A_ref(_layernorm(x, axis=-1), A_k_cache, A_v_cache, A_wq, A_wo)
    x = x + _B_ref(_layernorm(x, axis=-1), B_w1, B_b1, B_w2)
    x = x + _A_ref(_layernorm(x, axis=-1), A_k_cache, A_v_cache, A_wq, A_wo)
    x = x + _B_ref(_layernorm(x, axis=-1), B_w1, B_b1, B_w2)
    return x
```

```python
import functools
import jax
import jax.numpy as jnp
import numpy as np
import jax.experimental.pallas as pl
import jax.experimental.pallas.tpu as pltpu

D = 512
HQ, HKV, SK, DH = 32, 8, 65536, 128
REP = HQ // HKV
F = 1792
EPS = 1e-5
SCALE = 0.08837890625

BF = jnp.bfloat16
F32 = jnp.float32


def _ln(x):
    m = jnp.mean(x, axis=-1, keepdims=True)
    xc = x - m
    v = jnp.mean(xc * xc, axis=-1, keepdims=True)
    return xc * jax.lax.rsqrt(v + EPS)


def make_kernel(BK, NS, LOOK):
    NBG = SK // BK
    NB = HKV * NBG

    def kernel(x_ref, b1_ref, k_hbm, v_hbm, wq_hbm, wo_hbm, w1_hbm, w2_hbm, o_ref,
               kv, wq, wo, w1, w2, qs, sem, wsem):
        def kcopy(i, slot):
            return pltpu.make_async_copy(k_hbm.at[pl.ds(i * BK, BK)], kv.at[slot, 0], sem.at[slot])

        def vcopy(i, slot):
            return pltpu.make_async_copy(v_hbm.at[pl.ds(i * BK, BK)], kv.at[slot, 1], sem.at[slot])

        def start(i, slot):
            kcopy(i, slot).start()
            vcopy(i, slot).start()

        def wait(slot):
            kcopy(0, slot).wait()
            vcopy(0, slot).wait()

        cq = pltpu.make_async_copy(wq_hbm, wq, wsem.at[0])
        co = pltpu.make_async_copy(wo_hbm, wo, wsem.at[1])
        c1 = pltpu.make_async_copy(w1_hbm, w1, wsem.at[2])
        c2 = pltpu.make_async_copy(w2_hbm, w2, wsem.at[3])
        cq.start()
        for i in range(LOOK):
            start(i, i % NS)
        co.start()
        c1.start()
        c2.start()

        row = jax.lax.broadcasted_iota(jnp.int32, (8, DH), 0)

        def make_q(x):
            xn = _ln(x).astype(BF)
            for g in range(HKV):
                qq = jnp.dot(xn, wq[:, g * REP * DH:(g + 1) * REP * DH], preferred_element_type=F32)
                acc = jnp.zeros((8, DH), F32)
                for h in range(REP):
                    acc = jnp.where(row == h, qq[:, h * DH:(h + 1) * DH], acc)
                qs[g] = acc.astype(BF)

        def block(q, slot, m, l, acc):
            k = kv[slot, 0]
            v = kv[slot, 1]
            s = jax.lax.dot_general(q, k, (((1,), (1,)), ((), ())), preferred_element_type=F32) * SCALE
            m_new = jnp.maximum(m, jnp.max(s, axis=1, keepdims=True))
            p = jnp.exp(s - m_new)
            alpha = jnp.exp(m - m_new)
            l = l * alpha + jnp.sum(p, axis=1, keepdims=True)
            acc = acc * alpha + jnp.dot(p.astype(BF), v, preferred_element_type=F32)
            return m_new, l, acc

        def finalize(g, l, acc, y):
            o = (acc / l).astype(BF)
            for h in range(REP):
                oh = jnp.where(row == h, o, jnp.zeros_like(o))
                w = wo[pl.ds(pl.multiple_of((g * REP + h) * DH, DH), DH), :]
                y = y + jnp.dot(oh, w, preferred_element_type=F32)
            return y

        def ffn(x):
            xn = _ln(x).astype(BF)
            h = jnp.dot(xn, w1[...], preferred_element_type=F32) + b1_ref[...].astype(F32)
            sp = jnp.log1p(jnp.exp(-jnp.abs(h))) + jnp.maximum(h, 0.0)
            act = h * jnp.tanh(sp)
            return jnp.dot(act.astype(BF), w2[...], preferred_element_type=F32)

        def init():
            return (jnp.full((8, 1), -1e30, F32), jnp.zeros((8, 1), F32), jnp.zeros((8, DH), F32))

        x0 = jnp.broadcast_to(x_ref[...].astype(F32), (8, D))
        cq.wait()
        make_q(x0)

        def p1_group(g, y):
            q = qs[g]

            def body(j, carry):
                i = g * NBG + j
                slot = i % NS
                wait(slot)

                @pl.when(i + LOOK < NB)
                def _():
                    start(i + LOOK, (i + LOOK) % NS)
                return block(q, slot, *carry)
            m, l, acc = jax.lax.fori_loop(0, NBG, body, init())

            @pl.when(g == 0)
            def _():
                co.wait()
            return finalize(g, l, acc, y)

        y = jax.lax.fori_loop(0, HKV, p1_group, jnp.zeros((8, D), F32))
        x1 = x0 + jnp.sum(y, axis=0, keepdims=True)
        c1.wait()
        c2.wait()
        x2 = x1 + ffn(x1)
        make_q(x2)

        def p2_group(gg, y):
            g = HKV - 1 - gg
            q = qs[g]

            def body(jj, carry):
                i = g * NBG + (NBG - 1 - jj)
                slot = i % NS

                @pl.when(i < NB - NS)
                def _():
                    wait(slot)
                carry = block(q, slot, *carry)

                @pl.when(i - NS >= 0)
                def _():
                    start(i - NS, slot)
                return carry
            m, l, acc = jax.lax.fori_loop(0, NBG, body, init())
            return finalize(g, l, acc, y)

        y = jax.lax.fori_loop(0, HKV, p2_group, jnp.zeros((8, D), F32))
        x3 = x2 + jnp.sum(y, axis=0, keepdims=True)
        x4 = x3 + ffn(x3)
        o_ref[...] = x4[0:1, :].astype(o_ref.dtype)

    return kernel


def build(BK=4096, NS=58, LOOK=4):
    def fn(A_x, A_k_cache, A_v_cache, A_wq, A_wo, B_x, B_w1, B_b1, B_w2):
        x = A_x.reshape(1, D)
        b1 = B_b1.reshape(1, F)
        k = A_k_cache.reshape(HKV * SK, DH)
        v = A_v_cache.reshape(HKV * SK, DH)
        any_spec = pl.BlockSpec(memory_space=pl.ANY)
        vm = pl.BlockSpec(memory_space=pltpu.VMEM)
        out = pl.pallas_call(
            make_kernel(BK, NS, LOOK),
            out_shape=jax.ShapeDtypeStruct((1, D), A_x.dtype),
            in_specs=[vm, vm] + [any_spec] * 6,
            out_specs=vm,
            scratch_shapes=[
                pltpu.VMEM((NS, 2, BK, DH), BF),
                pltpu.VMEM((D, HQ * DH), BF),
                pltpu.VMEM((HQ * DH, D), BF),
                pltpu.VMEM((D, F), BF),
                pltpu.VMEM((F, D), BF),
                pltpu.VMEM((HKV, 8, DH), BF),
                pltpu.SemaphoreType.DMA((NS,)),
                pltpu.SemaphoreType.DMA((4,)),
            ],
            compiler_params=pltpu.CompilerParams(vmem_limit_bytes=128 * 1024 * 1024),
        )(x, b1, k, v, A_wq, A_wo, B_w1, B_w2)
        return out.reshape(1, 1, D)
    return jax.jit(fn)


_impl = build()


@jax.jit
def pallas_interleave_layers__gqa_block_cached__dense_activation_mish__decode_kernel(
    A_x: jax.Array,
    A_k_cache: jax.Array,
    A_v_cache: jax.Array,
    A_wq: jax.Array,
    A_wo: jax.Array,
    B_x: jax.Array,
    B_w1: jax.Array,
    B_b1: jax.Array,
    B_w2: jax.Array,
):
    return _impl(A_x, A_k_cache, A_v_cache, A_wq, A_wo, B_x, B_w1, B_b1, B_w2)
```

```python
import jax
import jax.numpy as jnp
import numpy as np
from jax import lax
import jax.experimental.pallas as pl
import jax.experimental.pallas.tpu as pltpu

D = 512
HQ, HKV, SK, DH = 32, 8, 65536, 128
REP = HQ // HKV
F = 1792
EPS = 1e-5
SCALE = 0.08837890625

BF = jnp.bfloat16
F32 = jnp.float32
I32 = jnp.int32

CH = 512
CR = CH // 2
CR12 = CR * 3 // 4
CR13 = CR * 13 // 16


def _c(x):
    return np.array([(x << 16) | x], np.uint32).view(np.int32)[0]


def _srl(x, n):
    return lax.shift_right_logical(x, np.int32(n))


def _shl(x, n):
    return lax.shift_left(x, np.int32(n))


def _enc12(x, kb):
    n = x.shape[0] // 4
    d = x - kb
    d0, d1, d2, d3 = (d[i * n:(i + 1) * n] for i in range(4))
    p0 = _shl(d3, 11) & _c(0x7800)
    p1 = _shl(d3, 7) & _c(0x7800)
    p2 = (_shl(d3, 3) & _c(0x3800)) | (_srl(d3, 1) & _c(0x4000))
    return jnp.concatenate([d0 | p0, d1 | p1, d2 | p2], axis=0)


def _dec12(h):
    n = h.shape[0] // 3
    h0, h1, h2 = h[0:n], h[n:2 * n], h[2 * n:3 * n]
    M, B = _c(0x87FF), _c(0x3800)
    w3 = ((_srl(h0, 11) & _c(0x000F)) | (_srl(h1, 7) & _c(0x00F0))
          | (_srl(h2, 3) & _c(0x0700)) | (_shl(h2, 1) & _c(0x8000)) | B)
    return jnp.concatenate([(h0 & M) | B, (h1 & M) | B, (h2 & M) | B, w3], axis=0)


def _enc13(x, kb):
    n = x.shape[0] // 16
    d = x - kb
    ds = [d[i * n:(i + 1) * n] for i in range(16)]
    SP = _c(0x7000)
    out = []
    for j in range(3):
        e = ds[13 + j]
        out.append(ds[4 * j + 0] | (_shl(e, 12) & SP))
        out.append(ds[4 * j + 1] | (_shl(e, 9) & SP))
        out.append(ds[4 * j + 2] | (_shl(e, 6) & SP))
        out.append(ds[4 * j + 3] | (_shl(e, 3) & SP))
    sg = ((_srl(ds[13], 3) & _c(0x1000)) | (_srl(ds[14], 2) & _c(0x2000))
          | (_srl(ds[15], 1) & _c(0x4000)))
    out.append(ds[12] | sg)
    return jnp.concatenate(out, axis=0)


def _dec13(h):
    n = h.shape[0] // 13
    hs = [h[i * n:(i + 1) * n] for i in range(13)]
    M, B = _c(0x8FFF), _c(0x3000)
    out = [(t & M) | B for t in hs]
    for j in range(3):
        w = ((_srl(hs[4 * j], 12) & _c(0x0007)) | (_srl(hs[4 * j + 1], 9) & _c(0x0038))
             | (_srl(hs[4 * j + 2], 6) & _c(0x01C0)) | (_srl(hs[4 * j + 3], 3) & _c(0x0E00)))
        out.append(w | (_shl(hs[12], 3 - j) & _c(0x8000)) | B)
    return jnp.concatenate(out, axis=0)


def _ln(x):
    m = jnp.mean(x, axis=-1, keepdims=True)
    xc = x - m
    v = jnp.mean(xc * xc, axis=-1, keepdims=True)
    return xc * lax.rsqrt(v + EPS)


def make_kernel(BK, S, NST, FORCE=0, DBG=0, SKEW=3):
    NBG = SK // BK
    NP = HKV * NBG
    TR = BK // 2
    NCH = BK // CH
    END = S * 2 * TR + NST

    def kernel(x_ref, b1_ref, k_hbm, v_hbm, wq_hbm, wo_hbm, w1_hbm, w2_hbm, o_ref,
               mem, wq, wo, w1, w2, qs, ms, ls, accs, ys,
               fmt, pos, bks, bvs, rl, sl, cnt, sem, wsem):
        k32 = k_hbm.bitcast(I32)
        v32 = v_hbm.bitcast(I32)

        def copies(pair, slot):
            return (pltpu.make_async_copy(k32.at[pl.ds(pair * TR, TR)], mem.at[pl.ds(slot * 2 * TR, TR)], sem.at[slot]),
                    pltpu.make_async_copy(v32.at[pl.ds(pair * TR, TR)], mem.at[pl.ds(slot * 2 * TR + TR, TR)], sem.at[slot]))

        def start(pair, slot):
            for c in copies(pair, slot):
                c.start()

        def wait(slot):
            for c in copies(0, slot):
                c.wait()

        cq = pltpu.make_async_copy(wq_hbm, wq, wsem.at[0])
        co = pltpu.make_async_copy(wo_hbm, wo, wsem.at[1])
        c1 = pltpu.make_async_copy(w1_hbm, w1, wsem.at[2])
        c2 = pltpu.make_async_copy(w2_hbm, w2, wsem.at[3])
        cq.start()
        for i in range(S):
            start(i, i)
        co.start()
        c1.start()
        c2.start()

        def zero(i, c):
            fmt[i] = 0
            pos[i] = 0
            bks[i] = 0
            bvs[i] = 0
            rl[i] = 0
            sl[i] = 0
            return c
        lax.fori_loop(0, NP, zero, 0)
        for g in range(HKV):
            cnt[g] = 0

        row = lax.broadcasted_iota(I32, (8, DH), 0)

        def make_q(x):
            xn = _ln(x).astype(BF)
            for g in range(HKV):
                qq = jnp.dot(xn, wq[:, g * REP * DH:(g + 1) * REP * DH], preferred_element_type=F32)
                acc = jnp.zeros((8, DH), F32)
                for h in range(REP):
                    acc = jnp.where(row == h, qq[:, h * DH:(h + 1) * DH], acc)
                qs[g] = acc.astype(BF)

        def reset_state():
            ms[...] = jnp.full(ms.shape, -1e30, F32)
            ls[...] = jnp.zeros(ls.shape, F32)
            accs[...] = jnp.zeros(accs.shape, F32)
            ys[...] = jnp.zeros(ys.shape, F32)

        def pow2(n):
            return pltpu.bitcast(_shl(jnp.full((8, 1), n + 127, I32), 23), F32)

        def attend(g, load_k, load_v, kscale, vscale):
            q = qs[g]
            ss = [lax.dot_general(q, pltpu.bitcast(load_k(c), BF), (((1,), (1,)), ((), ())),
                                  preferred_element_type=F32) for c in range(NCH)]
            s = jnp.concatenate(ss, axis=1) * kscale
            m_prev = ms[g][:, 0:1]
            m_new = jnp.maximum(m_prev, jnp.max(s, axis=1, keepdims=True))
            p = jnp.exp(s - m_new)
            alpha = jnp.exp(m_prev - m_new)
            l_new = alpha * ls[g][:, 0:1] + jnp.sum(p, axis=1, keepdims=True)
            pb = p.astype(BF)
            pv = None
            for c in range(NCH):
                t = jnp.dot(pb[:, c * CH:(c + 1) * CH], pltpu.bitcast(load_v(c), BF), preferred_element_type=F32)
                pv = t if pv is None else pv + t
            accs[g] = alpha * accs[g] + (pv if vscale is None else pv * vscale)
            ms[g] = jnp.broadcast_to(m_new, (8, DH))
            ls[g] = jnp.broadcast_to(l_new, (8, DH))

        def finalize(g):
            o = (accs[g] / ls[g]).astype(BF)
            y = ys[...]
            for h in range(REP):
                oh = jnp.where(row == h, o, jnp.zeros_like(o))
                w = wo[pl.ds(pl.multiple_of((g * REP + h) * DH, DH), DH), :]
                y = y + jnp.dot(oh, w, preferred_element_type=F32)
            ys[...] = y

        def ffn(x):
            xn = _ln(x).astype(BF)
            h = jnp.dot(xn, w1[...], preferred_element_type=F32)
            b = b1_ref[...].astype(F32)
            h = jnp.concatenate([h[:, j * DH:(j + 1) * DH] + b[j:j + 1, :] for j in range(F // DH)], axis=1)
            sp = jnp.log1p(jnp.exp(-jnp.abs(h))) + jnp.maximum(h, 0.0)
            act = h * jnp.tanh(sp)
            return jnp.dot(act.astype(BF), w2[...], preferred_element_type=F32)

        def raw_loader(off):
            return lambda c: mem[pl.ds(pl.multiple_of(off + c * CR, CR), CR), :]

        def exp_range(koff, trips):
            def body(c, carry):
                out = []
                for t, (mx, mn) in enumerate((carry[0:2], carry[2:4])):
                    x = mem[pl.ds(pl.multiple_of(koff + t * TR + c * CR, CR), CR), :]
                    hi = pltpu.bitcast(x & np.int32(0x7F800000), F32).reshape(CR // 8, 8, DH)
                    lo = pltpu.bitcast(_shl(x, 16) & np.int32(0x7F800000), F32).reshape(CR // 8, 8, DH)
                    out.append(jnp.maximum(mx, jnp.max(jnp.maximum(hi, lo), axis=0)))
                    out.append(jnp.minimum(mn, jnp.min(jnp.minimum(hi, lo), axis=0)))
                return tuple(out)
            z = jnp.zeros((8, DH), F32)
            big = jnp.full((8, DH), np.inf, F32)
            r = lax.fori_loop(0, trips, body, (z, big, z, big))
            e = [_srl(pltpu.bitcast(t, I32), 23).astype(F32) for t in r]
            return (jnp.max(e[0]).astype(I32), jnp.min(e[1]).astype(I32),
                    jnp.max(e[2]).astype(I32), jnp.min(e[3]).astype(I32))

        def fmt_of(mx, mn):
            ok = (mn >= 1) & (mx <= 254)
            w = mx - mn
            return jnp.where(ok & (w <= 15), 1, jnp.where(ok & (w <= 31), 2, 3))

        def rows_of(f):
            return jnp.where(f == 1, NCH * CR12, jnp.where(f == 2, NCH * CR13, NCH * CR))

        x0 = jnp.broadcast_to(x_ref[...].astype(F32), (8, D))
        reset_state()
        cq.wait()
        make_q(x0)

        def p1(i, carry):
            ptr, nr, ns = carry
            g = i // NBG
            slot = i % S
            koff = slot * 2 * TR
            voff = koff + TR
            wait(slot)
            attend(g, raw_loader(koff), raw_loader(voff), SCALE, None)
            live = i < NP - S
            room = live & (ptr + 2 * NCH * CR12 <= END)
            kmx, kmn, vmx, vmn = exp_range(koff, jnp.where(room, NCH, 0))
            f = jnp.maximum(fmt_of(kmx, kmn), fmt_of(vmx, vmn))
            if FORCE:
                f = jnp.maximum(f, FORCE)
            rows = rows_of(f)
            cache = live & (ptr + 2 * rows <= END)
            top = jnp.where(f == 1, 239, 223)
            bk = jnp.minimum(kmn, top)
            bv = jnp.minimum(vmn, top)

            def encode(enc, crows):
                def run():
                    for src, base, dst in ((koff, bk, ptr), (voff, bv, ptr + NCH * crows)):
                        kb = _shl(base, 7) | _shl(base, 23)
                        for c in range(NCH):
                            x = mem[pl.ds(pl.multiple_of(src + c * CR, CR), CR), :]
                            mem[pl.ds(pl.multiple_of(dst + c * crows, 8), crows), :] = enc(x, kb)
                return run

            pl.when(cache & (f == 1))(encode(_enc12, CR12))
            pl.when(cache & (f == 2))(encode(_enc13, CR13))
            pl.when(cache & (f == 3))(encode(lambda x, kb: x, CR))

            @pl.when(i + S < NP)
            def _():
                start(i + S, slot)

            @pl.when(cache)
            def _():
                fmt[i] = f
                pos[i] = ptr
                bks[i] = bk
                bvs[i] = bv
                rl[nr] = i

            @pl.when(live & jnp.logical_not(cache))
            def _():
                sl[ns] = i

            @pl.when(i % NBG == NBG - 1)
            def _():
                @pl.when(i == NBG - 1)
                def _():
                    co.wait()
                finalize(g)

            ci = cache.astype(I32)
            return ptr + 2 * rows * ci, nr + ci, ns + live.astype(I32) - ci

        _, nr, ns = lax.fori_loop(0, NP, p1, (jnp.int32(S * 2 * TR), jnp.int32(0), jnp.int32(0)))
        x1 = x0 + jnp.sum(ys[...], axis=0, keepdims=True)
        c1.wait()
        c2.wait()
        x2 = x1 + ffn(x1)
        reset_state()
        make_q(x2)
        if DBG == 1:
            o_ref[...] = (x2[0:1, :] + qs[0][0:1, :].astype(F32).sum()).astype(o_ref.dtype)
            return

        nring = ns + S
        span = jnp.maximum(nring - SKEW, 1)

        def p2(step, carry):
            t, r = carry
            ring = (t < nring) & ((r >= nr) | (t * nr <= r * span))
            slot = (NP - S + t) % S
            ring_pair = jnp.where(t < S, NP - S + t, sl[jnp.clip(t - S, 0, NP - 1)])
            res_pair = rl[jnp.minimum(r, NP - 1)]
            pair = jnp.where(ring, ring_pair, res_pair)
            f = jnp.where(ring, 3, fmt[res_pair])
            koff = jnp.where(ring, slot * 2 * TR, pos[res_pair])
            voff = koff + rows_of(f)
            g = pair // NBG

            @pl.when(ring & (t >= S))
            def _():
                wait(slot)

            def dec(decf, crows, bias):
                def run():
                    def loader(off):
                        return lambda c: decf(mem[pl.ds(pl.multiple_of(off + c * crows, 8), crows), :])
                    attend(g, loader(koff), loader(koff + NCH * crows),
                           SCALE * pow2(bks[res_pair] - bias), pow2(bvs[res_pair] - bias))
                return run

            pl.when(f == 1)(dec(_dec12, CR12, 112))
            pl.when(f == 2)(dec(_dec13, CR13, 96))

            @pl.when(f == 3)
            def _():
                attend(g, raw_loader(koff), raw_loader(voff), SCALE, None)

            @pl.when(ring & (t < ns))
            def _():
                start(sl[t], slot)

            done = cnt[g] + 1
            cnt[g] = done

            @pl.when(done == NBG)
            def _():
                finalize(g)

            ri = ring.astype(I32)
            return t + ri, r + 1 - ri

        lax.fori_loop(0, NP, p2, (jnp.int32(0), jnp.int32(0)))

        x3 = x2 + jnp.sum(ys[...], axis=0, keepdims=True)
        x4 = x3 + ffn(x3)
        o_ref[...] = x4[0:1, :].astype(o_ref.dtype)

    return kernel, NP, END


def build(BK=4096, S=2, NST=229000, FORCE=0, DBG=0, SKEW=3):
    def fn(A_x, A_k_cache, A_v_cache, A_wq, A_wo, B_x, B_w1, B_b1, B_w2):
        x = A_x.reshape(1, D)
        b1 = B_b1.reshape(F // DH, DH)
        k = A_k_cache.reshape(HKV * SK, DH)
        v = A_v_cache.reshape(HKV * SK, DH)
        any_spec = pl.BlockSpec(memory_space=pl.ANY)
        vm = pl.BlockSpec(memory_space=pltpu.VMEM)
        kern, NP, END = make_kernel(BK, S, NST, FORCE, DBG, SKEW)
        out = pl.pallas_call(
            kern,
            out_shape=jax.ShapeDtypeStruct((1, D), A_x.dtype),
            in_specs=[vm, vm] + [any_spec] * 6,
            out_specs=vm,
            scratch_shapes=[
                pltpu.VMEM((END, DH), I32),
                pltpu.VMEM((D, HQ * DH), BF),
                pltpu.VMEM((HQ * DH, D), BF),
                pltpu.VMEM((D, F), BF),
                pltpu.VMEM((F, D), BF),
                pltpu.VMEM((HKV, 8, DH), BF),
                pltpu.VMEM((HKV, 8, DH), F32),
                pltpu.VMEM((HKV, 8, DH), F32),
                pltpu.VMEM((HKV, 8, DH), F32),
                pltpu.VMEM((8, D), F32),
            ] + [pltpu.SMEM((NP,), I32)] * 6 + [pltpu.SMEM((HKV,), I32)] + [
                pltpu.SemaphoreType.DMA((S,)),
                pltpu.SemaphoreType.DMA((4,)),
            ],
            compiler_params=pltpu.CompilerParams(vmem_limit_bytes=128 * 1024 * 1024),
        )(x, b1, k, v, A_wq, A_wo, B_w1, B_w2)
        return out.reshape(1, 1, D)
    return jax.jit(fn)


_impl = build(BK=4096, S=3, NST=225000)


@jax.jit
def pallas_interleave_layers__gqa_block_cached__dense_activation_mish__decode_kernel(
    A_x: jax.Array,
    A_k_cache: jax.Array,
    A_v_cache: jax.Array,
    A_wq: jax.Array,
    A_wo: jax.Array,
    B_x: jax.Array,
    B_w1: jax.Array,
    B_b1: jax.Array,
    B_w2: jax.Array,
):
    return _impl(A_x, A_k_cache, A_v_cache, A_wq, A_wo, B_x, B_w1, B_b1, B_w2)
```

```python
import jax
import jax.numpy as jnp
import numpy as np
from jax import lax
import jax.experimental.pallas as pl
import jax.experimental.pallas.tpu as pltpu

D = 512
HQ, HKV, SK, DH = 32, 8, 65536, 128
REP = HQ // HKV
F = 1792
EPS = 1e-5
SCALE = 0.08837890625

BF = jnp.bfloat16
F32 = jnp.float32
I32 = jnp.int32

CH = 512
CR = CH // 2
CR12 = CR * 3 // 4
CR13 = CR * 13 // 16


def _c(x):
    return np.array([(x << 16) | x], np.uint32).view(np.int32)[0]


def _srl(x, n):
    return lax.shift_right_logical(x, np.int32(n))


def _shl(x, n):
    return lax.shift_left(x, np.int32(n))


def _enc12(x, kb):
    n = x.shape[0] // 4
    d = x - kb
    d0, d1, d2, d3 = (d[i * n:(i + 1) * n] for i in range(4))
    p0 = _shl(d3, 11) & _c(0x7800)
    p1 = _shl(d3, 7) & _c(0x7800)
    p2 = (_shl(d3, 3) & _c(0x3800)) | (_srl(d3, 1) & _c(0x4000))
    return jnp.concatenate([d0 | p0, d1 | p1, d2 | p2], axis=0)


def _dec12(h):
    n = h.shape[0] // 3
    h0, h1, h2 = h[0:n], h[n:2 * n], h[2 * n:3 * n]
    M, B = _c(0x87FF), _c(0x3800)
    w3 = ((_srl(h0, 11) & _c(0x000F)) | (_srl(h1, 7) & _c(0x00F0))
          | (_srl(h2, 3) & _c(0x0700)) | (_shl(h2, 1) & _c(0x8000)) | B)
    return jnp.concatenate([(h0 & M) | B, (h1 & M) | B, (h2 & M) | B, w3], axis=0)


def _enc13(x, kb):
    n = x.shape[0] // 16
    d = x - kb
    ds = [d[i * n:(i + 1) * n] for i in range(16)]
    SP = _c(0x7000)
    out = []
    for j in range(3):
        e = ds[13 + j]
        out.append(ds[4 * j + 0] | (_shl(e, 12) & SP))
        out.append(ds[4 * j + 1] | (_shl(e, 9) & SP))
        out.append(ds[4 * j + 2] | (_shl(e, 6) & SP))
        out.append(ds[4 * j + 3] | (_shl(e, 3) & SP))
    sg = ((_srl(ds[13], 3) & _c(0x1000)) | (_srl(ds[14], 2) & _c(0x2000))
          | (_srl(ds[15], 1) & _c(0x4000)))
    out.append(ds[12] | sg)
    return jnp.concatenate(out, axis=0)


def _dec13(h):
    n = h.shape[0] // 13
    hs = [h[i * n:(i + 1) * n] for i in range(13)]
    M, B = _c(0x8FFF), _c(0x3000)
    out = [(t & M) | B for t in hs]
    for j in range(3):
        w = ((_srl(hs[4 * j], 12) & _c(0x0007)) | (_srl(hs[4 * j + 1], 9) & _c(0x0038))
             | (_srl(hs[4 * j + 2], 6) & _c(0x01C0)) | (_srl(hs[4 * j + 3], 3) & _c(0x0E00)))
        out.append(w | (_shl(hs[12], 3 - j) & _c(0x8000)) | B)
    return jnp.concatenate(out, axis=0)


def _ln(x):
    m = jnp.mean(x, axis=-1, keepdims=True)
    xc = x - m
    v = jnp.mean(xc * xc, axis=-1, keepdims=True)
    return xc * lax.rsqrt(v + EPS)


def make_kernel(BK, S, NST, FORCE=0, DBG=0, SKEW=3, NSPLIT=32, DUNROLL=1, NSTR=1, PK=0, PERM=None):
    NBG = SK // BK
    NP = HKV * NBG
    TR = BK // 2
    NCH = BK // CH
    END = S * 2 * TR + NST

    def kernel(x_ref, b1_ref, k_hbm, v_hbm, wq_hbm, wo_hbm, w1_hbm, w2_hbm, o_ref,
               mem, wq, wo, w1, w2, qs, ms, ls, accs, ys,
               fmt, pos, bks, bvs, rl, sl, cnt, sem, wsem):
        k32 = k_hbm.bitcast(I32)
        v32 = v_hbm.bitcast(I32)

        SUB = TR // NSPLIT

        def start(pair, slot):
            if PERM is not None:
                pk, pv = PERM
                for a, b in zip(pk, pv):
                    src = pl.multiple_of(pair * TR, SUB)
                    dst = pl.multiple_of(slot * 2 * TR, SUB)
                    pltpu.make_async_copy(k32.at[pl.ds(src + a * SUB, SUB)], mem.at[pl.ds(dst + a * SUB, SUB)], sem.at[slot]).start(priority=PK)
                    pltpu.make_async_copy(v32.at[pl.ds(src + b * SUB, SUB)], mem.at[pl.ds(dst + TR + b * SUB, SUB)], sem.at[slot]).start(priority=1 - PK)
                return

            def body(j, c):
                for st in range(NSTR):
                    off = st * (TR // NSTR) + j * SUB
                    src = pl.multiple_of(pair * TR + off, SUB)
                    dst = pl.multiple_of(slot * 2 * TR + off, SUB)
                    pltpu.make_async_copy(k32.at[pl.ds(src, SUB)], mem.at[pl.ds(dst, SUB)], sem.at[slot]).start(priority=PK)
                    pltpu.make_async_copy(v32.at[pl.ds(src, SUB)], mem.at[pl.ds(dst + TR, SUB)], sem.at[slot]).start(priority=1 - PK)
                return c
            lax.fori_loop(0, NSPLIT // NSTR, body, 0, unroll=max(1, DUNROLL // NSTR))

        def wait(slot):
            whole = mem.at[pl.ds(pl.multiple_of(slot * 2 * TR, TR), 2 * TR)]
            pltpu.make_async_copy(whole, whole, sem.at[slot]).wait()

        cq = pltpu.make_async_copy(wq_hbm, wq, wsem.at[0])
        co = pltpu.make_async_copy(wo_hbm, wo, wsem.at[1])
        c1 = pltpu.make_async_copy(w1_hbm, w1, wsem.at[2])
        c2 = pltpu.make_async_copy(w2_hbm, w2, wsem.at[3])
        cq.start()
        lax.fori_loop(0, S, lambda i, c: (start(i, i), c)[1], 0)
        co.start()
        c1.start()
        c2.start()

        def zero(i, c):
            fmt[i] = 0
            pos[i] = 0
            bks[i] = 0
            bvs[i] = 0
            rl[i] = 0
            sl[i] = 0
            return c
        lax.fori_loop(0, NP, zero, 0)
        for g in range(HKV):
            cnt[g] = 0

        row = lax.broadcasted_iota(I32, (8, DH), 0)

        def make_q(x):
            xn = _ln(x).astype(BF)
            for g in range(HKV):
                qq = jnp.dot(xn, wq[:, g * REP * DH:(g + 1) * REP * DH], preferred_element_type=F32)
                acc = jnp.zeros((8, DH), F32)
                for h in range(REP):
                    acc = jnp.where(row == h, qq[:, h * DH:(h + 1) * DH], acc)
                qs[g] = acc.astype(BF)

        def reset_state():
            ms[...] = jnp.full(ms.shape, -1e30, F32)
            ls[...] = jnp.zeros(ls.shape, F32)
            accs[...] = jnp.zeros(accs.shape, F32)
            ys[...] = jnp.zeros(ys.shape, F32)

        def pow2(n):
            return pltpu.bitcast(_shl(jnp.full((8, 1), n + 127, I32), 23), F32)

        def attend(g, load_k, load_v, kscale, vscale):
            q = qs[g]
            ss = [lax.dot_general(q, pltpu.bitcast(load_k(c), BF), (((1,), (1,)), ((), ())),
                                  preferred_element_type=F32) for c in range(NCH)]
            s = jnp.concatenate(ss, axis=1) * kscale
            m_prev = ms[g][:, 0:1]
            m_new = jnp.maximum(m_prev, jnp.max(s, axis=1, keepdims=True))
            p = jnp.exp(s - m_new)
            alpha = jnp.exp(m_prev - m_new)
            l_new = alpha * ls[g][:, 0:1] + jnp.sum(p, axis=1, keepdims=True)
            pb = p.astype(BF)
            pv = None
            for c in range(NCH):
                t = jnp.dot(pb[:, c * CH:(c + 1) * CH], pltpu.bitcast(load_v(c), BF), preferred_element_type=F32)
                pv = t if pv is None else pv + t
            accs[g] = alpha * accs[g] + (pv if vscale is None else pv * vscale)
            ms[g] = jnp.broadcast_to(m_new, (8, DH))
            ls[g] = jnp.broadcast_to(l_new, (8, DH))

        def finalize(g):
            o = (accs[g] / ls[g]).astype(BF)
            y = ys[...]
            for h in range(REP):
                oh = jnp.where(row == h, o, jnp.zeros_like(o))
                w = wo[pl.ds(pl.multiple_of((g * REP + h) * DH, DH), DH), :]
                y = y + jnp.dot(oh, w, preferred_element_type=F32)
            ys[...] = y

        def ffn(x):
            xn = _ln(x).astype(BF)
            h = jnp.dot(xn, w1[...], preferred_element_type=F32)
            b = b1_ref[...].astype(F32)
            h = jnp.concatenate([h[:, j * DH:(j + 1) * DH] + b[j:j + 1, :] for j in range(F // DH)], axis=1)
            sp = jnp.log1p(jnp.exp(-jnp.abs(h))) + jnp.maximum(h, 0.0)
            act = h * jnp.tanh(sp)
            return jnp.dot(act.astype(BF), w2[...], preferred_element_type=F32)

        def raw_loader(off):
            return lambda c: mem[pl.ds(pl.multiple_of(off + c * CR, CR), CR), :]

        def exp_range(koff, trips):
            def body(c, carry):
                out = []
                for t, (mx, mn) in enumerate((carry[0:2], carry[2:4])):
                    x = mem[pl.ds(pl.multiple_of(koff + t * TR + c * CR, CR), CR), :]
                    hi = pltpu.bitcast(x & np.int32(0x7F800000), F32).reshape(CR // 8, 8, DH)
                    lo = pltpu.bitcast(_shl(x, 16) & np.int32(0x7F800000), F32).reshape(CR // 8, 8, DH)
                    out.append(jnp.maximum(mx, jnp.max(jnp.maximum(hi, lo), axis=0)))
                    out.append(jnp.minimum(mn, jnp.min(jnp.minimum(hi, lo), axis=0)))
                return tuple(out)
            z = jnp.zeros((8, DH), F32)
            big = jnp.full((8, DH), np.inf, F32)
            r = lax.fori_loop(0, trips, body, (z, big, z, big))
            e = [_srl(pltpu.bitcast(t, I32), 23).astype(F32) for t in r]
            return (jnp.max(e[0]).astype(I32), jnp.min(e[1]).astype(I32),
                    jnp.max(e[2]).astype(I32), jnp.min(e[3]).astype(I32))

        def fmt_of(mx, mn):
            ok = (mn >= 1) & (mx <= 254)
            w = mx - mn
            return jnp.where(ok & (w <= 15), 1, jnp.where(ok & (w <= 31), 2, 3))

        def rows_of(f):
            return jnp.where(f == 1, NCH * CR12, jnp.where(f == 2, NCH * CR13, NCH * CR))

        x0 = jnp.broadcast_to(x_ref[...].astype(F32), (8, D))
        reset_state()
        cq.wait()
        make_q(x0)

        def p1(i, carry):
            ptr, nr, ns = carry
            g = i // NBG
            slot = i % S
            koff = slot * 2 * TR
            voff = koff + TR
            wait(slot)
            attend(g, raw_loader(koff), raw_loader(voff), SCALE, None)
            live = i < NP - S
            room = live & (ptr + 2 * NCH * CR12 <= END)
            kmx, kmn, vmx, vmn = exp_range(koff, jnp.where(room, NCH, 0))
            f = jnp.maximum(fmt_of(kmx, kmn), fmt_of(vmx, vmn))
            if FORCE:
                f = jnp.maximum(f, FORCE)
            rows = rows_of(f)
            cache = live & (ptr + 2 * rows <= END)
            top = jnp.where(f == 1, 239, 223)
            bk = jnp.minimum(kmn, top)
            bv = jnp.minimum(vmn, top)

            def encode(enc, crows):
                def run():
                    for src, base, dst in ((koff, bk, ptr), (voff, bv, ptr + NCH * crows)):
                        kb = _shl(base, 7) | _shl(base, 23)
                        for c in range(NCH):
                            x = mem[pl.ds(pl.multiple_of(src + c * CR, CR), CR), :]
                            mem[pl.ds(pl.multiple_of(dst + c * crows, 8), crows), :] = enc(x, kb)
                return run

            pl.when(cache & (f == 1))(encode(_enc12, CR12))
            pl.when(cache & (f == 2))(encode(_enc13, CR13))
            pl.when(cache & (f == 3))(encode(lambda x, kb: x, CR))

            @pl.when(i + S < NP)
            def _():
                start(i + S, slot)

            @pl.when(cache)
            def _():
                fmt[i] = f
                pos[i] = ptr
                bks[i] = bk
                bvs[i] = bv
                rl[nr] = i

            @pl.when(live & jnp.logical_not(cache))
            def _():
                sl[ns] = i

            @pl.when(i % NBG == NBG - 1)
            def _():
                @pl.when(i == NBG - 1)
                def _():
                    co.wait()
                finalize(g)

            ci = cache.astype(I32)
            return ptr + 2 * rows * ci, nr + ci, ns + live.astype(I32) - ci

        _, nr, ns = lax.fori_loop(0, NP, p1, (jnp.int32(S * 2 * TR), jnp.int32(0), jnp.int32(0)))
        x1 = x0 + jnp.sum(ys[...], axis=0, keepdims=True)
        c1.wait()
        c2.wait()
        x2 = x1 + ffn(x1)
        reset_state()
        make_q(x2)
        if DBG == 1:
            o_ref[...] = (x2[0:1, :] + qs[0][0:1, :].astype(F32).sum()).astype(o_ref.dtype)
            return

        nring = ns + S
        span = jnp.maximum(nring - SKEW, 1)

        def p2(step, carry):
            t, r = carry
            ring = (t < nring) & ((r >= nr) | (t * nr <= r * span))
            slot = (NP - S + t) % S
            ring_pair = jnp.where(t < S, NP - S + t, sl[jnp.clip(t - S, 0, NP - 1)])
            res_pair = rl[jnp.minimum(r, NP - 1)]
            pair = jnp.where(ring, ring_pair, res_pair)
            f = jnp.where(ring, 3, fmt[res_pair])
            koff = jnp.where(ring, slot * 2 * TR, pos[res_pair])
            voff = koff + rows_of(f)
            g = pair // NBG

            @pl.when(ring & (t >= S))
            def _():
                wait(slot)

            def dec(decf, crows, bias):
                def run():
                    def loader(off):
                        return lambda c: decf(mem[pl.ds(pl.multiple_of(off + c * crows, 8), crows), :])
                    attend(g, loader(koff), loader(koff + NCH * crows),
                           SCALE * pow2(bks[res_pair] - bias), pow2(bvs[res_pair] - bias))
                return run

            pl.when(f == 1)(dec(_dec12, CR12, 112))
            pl.when(f == 2)(dec(_dec13, CR13, 96))

            @pl.when(f == 3)
            def _():
                attend(g, raw_loader(koff), raw_loader(voff), SCALE, None)

            @pl.when(ring & (t < ns))
            def _():
                start(sl[t], slot)

            done = cnt[g] + 1
            cnt[g] = done

            @pl.when(done == NBG)
            def _():
                finalize(g)

            ri = ring.astype(I32)
            return t + ri, r + 1 - ri

        lax.fori_loop(0, NP, p2, (jnp.int32(0), jnp.int32(0)))

        x3 = x2 + jnp.sum(ys[...], axis=0, keepdims=True)
        x4 = x3 + ffn(x3)
        o_ref[...] = x4[0:1, :].astype(o_ref.dtype)

    return kernel, NP, END


def build(BK=4096, S=2, NST=229000, FORCE=0, DBG=0, SKEW=3, NSPLIT=32, DUNROLL=4, NOBC=True, NSTR=1, PK=0, PERM=None):
    def fn(A_x, A_k_cache, A_v_cache, A_wq, A_wo, B_x, B_w1, B_b1, B_w2):
        x = A_x.reshape(1, D)
        b1 = B_b1.reshape(F // DH, DH)
        k = A_k_cache.reshape(HKV * SK, DH)
        v = A_v_cache.reshape(HKV * SK, DH)
        any_spec = pl.BlockSpec(memory_space=pl.ANY)
        vm = pl.BlockSpec(memory_space=pltpu.VMEM)
        kern, NP, END = make_kernel(BK, S, NST, FORCE, DBG, SKEW, NSPLIT, DUNROLL, NSTR, PK, PERM)
        out = pl.pallas_call(
            kern,
            out_shape=jax.ShapeDtypeStruct((1, D), A_x.dtype),
            in_specs=[vm, vm] + [any_spec] * 6,
            out_specs=vm,
            scratch_shapes=[
                pltpu.VMEM((END, DH), I32),
                pltpu.VMEM((D, HQ * DH), BF),
                pltpu.VMEM((HQ * DH, D), BF),
                pltpu.VMEM((D, F), BF),
                pltpu.VMEM((F, D), BF),
                pltpu.VMEM((HKV, 8, DH), BF),
                pltpu.VMEM((HKV, 8, DH), F32),
                pltpu.VMEM((HKV, 8, DH), F32),
                pltpu.VMEM((HKV, 8, DH), F32),
                pltpu.VMEM((8, D), F32),
            ] + [pltpu.SMEM((NP,), I32)] * 6 + [pltpu.SMEM((HKV,), I32)] + [
                pltpu.SemaphoreType.DMA((S,)),
                pltpu.SemaphoreType.DMA((4,)),
            ],
            compiler_params=pltpu.CompilerParams(vmem_limit_bytes=128 * 1024 * 1024, disable_bounds_checks=NOBC),
        )(x, b1, k, v, A_wq, A_wo, B_w1, B_w2)
        return out.reshape(1, 1, D)
    return jax.jit(fn)


_impl = build(BK=4096, S=3, NST=225000, NSTR=2)


@jax.jit
def pallas_interleave_layers__gqa_block_cached__dense_activation_mish__decode_kernel(
    A_x: jax.Array,
    A_k_cache: jax.Array,
    A_v_cache: jax.Array,
    A_wq: jax.Array,
    A_wo: jax.Array,
    B_x: jax.Array,
    B_w1: jax.Array,
    B_b1: jax.Array,
    B_w2: jax.Array,
):
    return _impl(A_x, A_k_cache, A_v_cache, A_wq, A_wo, B_x, B_w1, B_b1, B_w2)
```

```python
import jax
import jax.numpy as jnp
import numpy as np
from jax import lax
import jax.experimental.pallas as pl
import jax.experimental.pallas.tpu as pltpu

D = 512
HQ, HKV, SK, DH = 32, 8, 65536, 128
REP = HQ // HKV
F = 1792
EPS = 1e-5
SCALE = 0.08837890625

BF = jnp.bfloat16
F32 = jnp.float32
I32 = jnp.int32

BK = 4096
TR = BK // 2
NBG = SK // BK
NP = HKV * NBG
CH = 512
NCH = BK // CH
CR = CH // 2
CR12 = CR * 3 // 4
CR13 = CR * 13 // 16
PACK12, PACK13, RAW = 1, 2, 3

SUB = 64
S = 3
END = 261000
PARTS = 4
SKEW = 3
WI, WJOBS, LATE = 5, 26, 2

WQ_OFF, WO_OFF, W1_OFF, W2_OFF = 0, HQ * CR, 2 * HQ * CR, 2 * HQ * CR + (F // DH) * CR
W2R = F // 2
WROWS = W2_OFF + (D // DH) * W2R


def _c(x):
    return np.array([(x << 16) | x], np.uint32).view(np.int32)[0]


def _srl(x, n):
    return lax.shift_right_logical(x, np.int32(n))


def _shl(x, n):
    return lax.shift_left(x, np.int32(n))


def _pack12(x, base):
    n = x.shape[0] // 4
    d = x - (_shl(base, 7) | _shl(base, 23))
    d0, d1, d2, d3 = (d[i * n:(i + 1) * n] for i in range(4))
    p0 = _shl(d3, 11) & _c(0x7800)
    p1 = _shl(d3, 7) & _c(0x7800)
    p2 = (_shl(d3, 3) & _c(0x3800)) | (_srl(d3, 1) & _c(0x4000))
    return jnp.concatenate([d0 | p0, d1 | p1, d2 | p2], axis=0), (d0 | d1) | (d2 | d3)


def _unpack12(h):
    n = h.shape[0] // 3
    h0, h1, h2 = h[0:n], h[n:2 * n], h[2 * n:3 * n]
    keep, bias = _c(0x87FF), _c(0x3800)
    w3 = ((_srl(h0, 11) & _c(0x000F)) | (_srl(h1, 7) & _c(0x00F0))
          | (_srl(h2, 3) & _c(0x0700)) | (_shl(h2, 1) & _c(0x8000)) | bias)
    return jnp.concatenate([(h0 & keep) | bias, (h1 & keep) | bias, (h2 & keep) | bias, w3], axis=0)


def _pack13(x, base):
    n = x.shape[0] // 16
    d = x - (_shl(base, 7) | _shl(base, 23))
    ds = [d[i * n:(i + 1) * n] for i in range(16)]
    out = []
    for j in range(3):
        for t in range(4):
            out.append(ds[4 * j + t] | (_shl(ds[13 + j], 12 - 3 * t) & _c(0x7000)))
    out.append(ds[12] | (_srl(ds[13], 3) & _c(0x1000)) | (_srl(ds[14], 2) & _c(0x2000))
               | (_srl(ds[15], 1) & _c(0x4000)))
    return jnp.concatenate(out, axis=0)


def _unpack13(h):
    n = h.shape[0] // 13
    hs = [h[i * n:(i + 1) * n] for i in range(13)]
    keep, bias = _c(0x8FFF), _c(0x3000)
    out = [(t & keep) | bias for t in hs]
    for j in range(3):
        w = (_shl(hs[12], 3 - j) & _c(0x8000)) | bias
        for t in range(4):
            w = w | (_srl(hs[4 * j + t], 12 - 3 * t) & _c(0x0007 << (3 * t)))
        out.append(w)
    return jnp.concatenate(out, axis=0)


def _layernorm(x):
    m = jnp.mean(x, axis=-1, keepdims=True)
    xc = x - m
    v = jnp.mean(xc * xc, axis=-1, keepdims=True)
    return xc * lax.rsqrt(v + EPS)


def _pow2(n):
    return pltpu.bitcast(_shl(jnp.full((8, 1), n + 127, I32), 23), F32)


def _make_kernel():
    STORE0 = S * 2 * TR
    TMP = STORE0 + 16 * 2 * TR * 2
    assert TMP + WROWS <= END - WROWS and STORE0 + (WI + WJOBS) * 2 * TR <= TMP
    assert LATE * NBG - 1 <= WI + WJOBS and WI + WJOBS + LATE <= (LATE + 1) * NBG - 1

    def kernel(x_ref, b1_ref, k_hbm, v_hbm, wq_hbm, wo_hbm, w1_hbm, w2_hbm, o_ref,
               mem, qs, ms, ls, accs, ys, fo,
               fmt, pos, bks, bvs, rl, sl, cnt, wmeta, flag, sem, wsem):
        k32, v32 = k_hbm.bitcast(I32), v_hbm.bitcast(I32)

        def rows(start, n, align=8, clamp=True):
            if clamp:
                start = jnp.clip(start, 0, END - n)
            return pl.ds(pl.multiple_of(start, align), n)

        def start_pair(pair, slot):
            pair = jnp.clip(pair, 0, NP - 1)

            def body(j, c):
                for half in range(2):
                    off = half * (TR // 2) + (j + half) % (TR // 2 // SUB) * SUB
                    src = pl.ds(pl.multiple_of(pair * TR + off, SUB), SUB)
                    dst = slot * 2 * TR + off
                    pltpu.make_async_copy(k32.at[src], mem.at[rows(dst, SUB, SUB, False)], sem.at[slot]).start(priority=0)
                    pltpu.make_async_copy(v32.at[src], mem.at[rows(dst + TR, SUB, SUB, False)], sem.at[slot]).start(priority=1)
                return c
            lax.fori_loop(0, TR // 2 // SUB, body, 0, unroll=2)

        def wait_pair(slot):
            whole = mem.at[rows(slot * 2 * TR, 2 * TR, TR)]
            pltpu.make_async_copy(whole, whole, sem.at[slot]).wait()

        def col(j):
            return pl.ds(pl.multiple_of(j * DH, DH), DH)

        def start_weight(m):
            wq32, wo32, w132, w232 = (r.bitcast(I32) for r in (wq_hbm, wo_hbm, w1_hbm, w2_hbm))
            n, src, dst = (
                (HQ, lambda c: wq32.at[:, col(c)], lambda c: rows(TMP + WQ_OFF + c * CR, CR, CR)),
                (HQ, lambda c: wo32.at[pl.ds(pl.multiple_of(c // REP * CR, CR), CR), col(c % REP)],
                 lambda c: rows(TMP + WO_OFF + c * CR, CR, CR)),
                (F // DH, lambda c: w132.at[:, col(c)], lambda c: rows(TMP + W1_OFF + c * CR, CR, CR)),
                (D // DH, lambda c: w232.at[:, col(c)], lambda c: rows(TMP + W2_OFF + c * W2R, W2R)),
            )[m]

            def body(c2, carry):
                for p in range(2):
                    c = 2 * c2 + p
                    pltpu.make_async_copy(src(c), mem.at[dst(c)], wsem.at[m]).start(priority=p)
                return carry
            lax.fori_loop(0, n // 2, body, 0)

        def wait_weight(m):
            off, n = ((WQ_OFF, HQ * CR), (WO_OFF, HQ * CR), (W1_OFF, W2_OFF - W1_OFF), (W2_OFF, WROWS - W2_OFF))[m]
            whole = mem.at[pl.ds(TMP + off, n)]
            pltpu.make_async_copy(whole, whole, wsem.at[m]).wait()

        start_weight(0)
        lax.fori_loop(0, S, lambda i, c: (start_pair(i, i), c)[1], 0)
        for m in (1, 2, 3):
            start_weight(m)

        def clear(i, c):
            for ref in (fmt, pos, bks, bvs, rl, sl):
                ref[i] = 0
            return c
        lax.fori_loop(0, NP, clear, 0)
        for g in range(HKV):
            cnt[g] = 0

        head = lax.broadcasted_iota(I32, (8, DH), 0)

        def weight_loader(wbase, form, off, nrows):
            if form == RAW:
                return lambda c: pltpu.bitcast(mem[rows(wbase + off + c * nrows, nrows), :], BF)
            prow = nrows * 3 // 4
            return lambda c: pltpu.bitcast(_unpack12(mem[rows(wbase + off * 3 // 4 + c * prow, prow), :]), BF)

        def scaled(y, form, m):
            return y if form == RAW else y * _pow2(wmeta[1 + m] - 112)

        def make_q(x, wbase, form):
            xn = _layernorm(x).astype(BF)
            load = weight_loader(wbase, form, WQ_OFF, CR)
            for g in range(HKV):
                q = jnp.zeros((8, DH), F32)
                for h in range(REP):
                    q = jnp.where(head == h, jnp.dot(xn, load(g * REP + h), preferred_element_type=F32), q)
                qs[g] = scaled(q, form, 0).astype(BF)

        def project_out(g, wbase, form):
            o = (accs[g] / ls[g]).astype(BF)
            lhs = jnp.concatenate([jnp.where(head == h, o, jnp.zeros_like(o)) for h in range(REP)], axis=1)
            load = weight_loader(wbase, form, WO_OFF, CR)
            y = jnp.concatenate([jnp.dot(lhs, load(g * REP + j), preferred_element_type=F32)
                                 for j in range(D // DH)], axis=1)
            ys[...] += scaled(y, form, 1)

        def ffn(x, wbase, form):
            xn = _layernorm(x).astype(BF)
            load1 = weight_loader(wbase, form, W1_OFF, CR)
            load2 = weight_loader(wbase, form, W2_OFF, W2R)
            b = b1_ref[...].astype(F32)
            h = jnp.concatenate([scaled(jnp.dot(xn, load1(j), preferred_element_type=F32), form, 2) + b[j:j + 1, :]
                                 for j in range(F // DH)], axis=1)
            softplus = jnp.log1p(jnp.exp(-jnp.abs(h))) + jnp.maximum(h, 0.0)
            act = (h * jnp.tanh(softplus)).astype(BF)
            y = jnp.concatenate([jnp.dot(act, load2(j), preferred_element_type=F32) for j in range(D // DH)], axis=1)
            fo[...] = scaled(y, form, 3)

        def with_weights(fn, *args):
            for form in (PACK12, RAW):
                pl.when(wmeta[0] == form)(lambda form=form: fn(*args, END - (WROWS if form == RAW else WROWS * 3 // 4), form))

        def reset_state():
            ms[...] = jnp.full(ms.shape, -np.inf, F32)
            ls[...] = jnp.zeros(ls.shape, F32)
            accs[...] = jnp.zeros(accs.shape, F32)
            ys[...] = jnp.zeros(ys.shape, F32)

        def attend(g, load_k, load_v, kscale, vscale):
            q = qs[g]
            per = NCH // PARTS
            scores = [jnp.concatenate(
                [lax.dot_general(q, pltpu.bitcast(load_k(c), BF), (((1,), (1,)), ((), ())), preferred_element_type=F32)
                 for c in range(part * per, (part + 1) * per)], axis=1) * kscale for part in range(PARTS)]
            m, l, acc = ms[g][:, 0:1], ls[g][:, 0:1], accs[g]
            for part, s in enumerate(scores):
                m_new = jnp.maximum(m, jnp.max(s, axis=1, keepdims=True))
                p = jnp.exp(s - m_new)
                alpha = jnp.exp(m - m_new)
                l = alpha * l + jnp.sum(p, axis=1, keepdims=True)
                pb = p.astype(BF)
                pv = None
                for c in range(per):
                    t = jnp.dot(pb[:, c * CH:(c + 1) * CH], pltpu.bitcast(load_v(part * per + c), BF),
                                preferred_element_type=F32)
                    pv = t if pv is None else pv + t
                acc = alpha * acc + (pv if vscale is None else pv * vscale)
                m = m_new
            accs[g] = acc
            ms[g] = jnp.broadcast_to(m, (8, DH))
            ls[g] = jnp.broadcast_to(l, (8, DH))

        def raw_loader(off):
            return lambda c: mem[rows(off + c * CR, CR, CR), :]

        def exp_range(offs, trips):
            def body(c, carry):
                out = []
                for t, off in enumerate(offs):
                    x = mem[rows(off + c * CR, CR, CR), :]
                    hi = pltpu.bitcast(x & np.int32(0x7F800000), F32).reshape(CR // 8, 8, DH)
                    lo = pltpu.bitcast(_shl(x, 16) & np.int32(0x7F800000), F32).reshape(CR // 8, 8, DH)
                    out.append(jnp.maximum(carry[2 * t], jnp.max(jnp.maximum(hi, lo), axis=0)))
                    out.append(jnp.minimum(carry[2 * t + 1], jnp.min(jnp.minimum(hi, lo), axis=0)))
                return tuple(out)
            init = (jnp.zeros((8, DH), F32), jnp.full((8, DH), np.inf, F32)) * len(offs)
            r = lax.fori_loop(0, trips, body, init)
            e = [_srl(pltpu.bitcast(t, I32), 23).astype(F32) for t in r]
            return [(jnp.max(e[2 * t]).astype(I32), jnp.min(e[2 * t + 1]).astype(I32)) for t in range(len(offs))]

        def fits(mx, mn, width):
            return (mn >= 1) & (mx <= 254) & (mx - mn < width)

        def rows_of(f):
            return jnp.where(f == PACK12, NCH * CR12, jnp.where(f == PACK13, NCH * CR13, NCH * CR))

        def park_weights(job):
            @pl.when(job == 0)
            def _():
                for m in (1, 2, 3):
                    wait_weight(m)
                for m in range(4):
                    wmeta[1 + m] = 255
                    wmeta[5 + m] = 0

            @pl.when(job < 12)
            def _():
                m = jnp.where(job < 8, job // 4, job // 2 - 2)
                first_chunk = jnp.where(job < 8, job * 8, 2 * HQ + (job - 8) * 7)
                (mx, mn), = exp_range([TMP + first_chunk * CR], jnp.where(job < 8, 8, 7))
                wmeta[1 + m] = jnp.minimum(wmeta[1 + m], mn)
                wmeta[5 + m] = jnp.maximum(wmeta[5 + m], mx)

            @pl.when(job == 12)
            def _():
                ok = jnp.bool_(True)
                for m in range(4):
                    ok = ok & fits(wmeta[5 + m], wmeta[1 + m], 16)
                    wmeta[1 + m] = jnp.minimum(wmeta[1 + m], 239)
                wmeta[0] = jnp.where(ok, PACK12, RAW)

            def move(form):
                wbase = END - (WROWS if form == RAW else WROWS * 3 // 4)
                enc = (lambda x, base: x) if form == RAW else (lambda x, base: _pack12(x, base)[0])
                num, den = (1, 1) if form == RAW else (3, 4)

                @pl.when(job < 22)
                def _():
                    def narrow(c, carry):
                        m = jnp.where(c < HQ, 0, jnp.where(c < 2 * HQ, 1, 2))
                        mem[rows(wbase + c * (CR * num // den), CR * num // den), :] = enc(
                            mem[rows(TMP + c * CR, CR, CR), :], wmeta[1 + m])
                        return carry
                    lax.fori_loop((job - 12) * 8, jnp.minimum((job - 11) * 8, W2_OFF // CR), narrow, 0)

                @pl.when(job >= 22)
                def _():
                    c = job - 22
                    mem[rows(wbase + (W2_OFF + c * W2R) * num // den, W2R * num // den), :] = enc(
                        mem[rows(TMP + W2_OFF + c * W2R, W2R), :], wmeta[4])

            @pl.when(job >= 12)
            def _():
                for form in (PACK12, RAW):
                    pl.when(wmeta[0] == form)(lambda form=form: move(form))

        x0 = jnp.broadcast_to(x_ref[...].astype(F32), (8, D))
        reset_state()
        wait_weight(0)
        make_q(x0, TMP, RAW)

        def first(i, carry):
            ptr, nr, ns, pf, pbk, pbv = carry
            g = i // NBG
            slot = i % S
            koff = slot * 2 * TR
            voff = koff + TR
            wait_pair(slot)
            attend(g, raw_loader(koff), raw_loader(voff), SCALE, None)

            @pl.when((i >= WI) & (i < WI + WJOBS))
            def _():
                park_weights(i - WI)

            live = i < NP - S
            limit = END - jnp.where(wmeta[0] == PACK12, WROWS * 3 // 4, WROWS)
            room = live & (ptr + 2 * NCH * CR12 <= limit)

            def attempt(state):
                _, exact, f, bk, bv, _ = state
                (kmx, kmn), (vmx, vmn) = exp_range([koff, voff], jnp.where(room & exact, NCH, 0))
                fe = jnp.where(fits(kmx, kmn, 16) & fits(vmx, vmn, 16), PACK12,
                               jnp.where(fits(kmx, kmn, 32) & fits(vmx, vmn, 32), PACK13, RAW))
                top, width = jnp.where(fe == PACK12, 239, 223), jnp.where(fe == PACK12, 16, 32)

                def centred(mx, mn):
                    return jnp.clip(mn - (width - 1 - (mx - mn)) // 2, 1, top)
                f = jnp.where(exact, fe, f)
                bk = jnp.where(exact, centred(kmx, kmn), bk)
                bv = jnp.where(exact, centred(vmx, vmn), bv)
                park = live & (ptr + 2 * rows_of(f) <= limit)
                flag[0] = 0

                def encode(enc, crows, check):
                    def run():
                        bad = None
                        for src, base, dst in ((koff, bk, ptr), (voff, bv, ptr + NCH * crows)):
                            for c in range(NCH):
                                y = enc(mem[rows(src + c * CR, CR, CR), :], base)
                                if check:
                                    y, e = y
                                    bad = e if bad is None else bad | e
                                mem[rows(dst + c * crows, crows), :] = y
                        if check:
                            bad = (bad & _c(0x7800)).reshape(-1, 8, DH)
                            flag[0] = jnp.max(jnp.max((bad != 0).astype(F32), axis=0)).astype(I32)
                    return run
                pl.when(park & (f == PACK12))(encode(_pack12, CR12, True))
                pl.when(park & (f == PACK13))(encode(_pack13, CR13, False))
                pl.when(park & (f == RAW))(encode(lambda x, base: x, CR, False))
                return (flag[0] != 0) & jnp.logical_not(exact), jnp.bool_(True), f, bk, bv, park

            _, _, f, bk, bv, park = lax.while_loop(
                lambda state: state[0], attempt,
                (jnp.bool_(True), pf != PACK12, pf, pbk, pbv, jnp.bool_(False)))
            size = 2 * rows_of(f)

            @pl.when(i + S < NP)
            def _():
                start_pair(i + S, slot)

            @pl.when(park)
            def _():
                fmt[i] = f
                pos[i] = ptr
                bks[i] = bk
                bvs[i] = bv
                rl[jnp.minimum(nr, NP - 1)] = i

            @pl.when(live & jnp.logical_not(park))
            def _():
                sl[jnp.minimum(ns, NP - 1)] = i

            done = (i % NBG == NBG - 1) & (i >= LATE * NBG)

            @pl.when(done | ((i >= WI + WJOBS) & (i < WI + WJOBS + LATE)))
            def _():
                with_weights(project_out, jnp.where(done, g, jnp.clip(i - WI - WJOBS, 0, HKV - 1)))

            parked = park.astype(I32)
            return ptr + size * parked, nr + parked, ns + live.astype(I32) - parked, f, bk, bv

        wmeta[0] = RAW
        _, nr, ns, _, _, _ = lax.fori_loop(0, NP, first, tuple(jnp.int32(v) for v in (STORE0, 0, 0, RAW, 1, 1)))
        x1 = x0 + jnp.sum(ys[...], axis=0, keepdims=True)
        with_weights(ffn, x1)
        x2 = x1 + fo[...]
        reset_state()
        with_weights(make_q, x2)
        nring = ns + S
        span = jnp.maximum(nring - SKEW, 1)

        def second(step, carry):
            t, r = carry
            ring = (t < nring) & ((r >= nr) | (t * nr <= r * span))
            slot = (NP - S + t) % S
            ring_pair = jnp.where(t < S, NP - S + t, sl[jnp.clip(t - S, 0, NP - 1)])
            res_pair = jnp.clip(rl[jnp.minimum(r, NP - 1)], 0, NP - 1)
            pair = jnp.clip(jnp.where(ring, ring_pair, res_pair), 0, NP - 1)
            f = jnp.where(ring, RAW, fmt[res_pair])
            koff = jnp.where(ring, slot * 2 * TR, pos[res_pair])
            g = pair // NBG

            @pl.when(ring & (t >= S))
            def _():
                wait_pair(slot)

            def packed(unpack, crows, bias):
                def run():
                    def loader(off):
                        return lambda c: unpack(mem[rows(off + c * crows, crows), :])
                    attend(g, loader(koff), loader(koff + NCH * crows),
                           SCALE * _pow2(bks[res_pair] - bias), _pow2(bvs[res_pair] - bias))
                return run
            pl.when(f == PACK12)(packed(_unpack12, CR12, 112))
            pl.when(f == PACK13)(packed(_unpack13, CR13, 96))

            @pl.when(f == RAW)
            def _():
                attend(g, raw_loader(koff), raw_loader(koff + TR), SCALE, None)

            @pl.when(ring & (t < ns))
            def _():
                start_pair(sl[jnp.minimum(t, NP - 1)], slot)

            done = cnt[g] + 1
            cnt[g] = done

            @pl.when(done == NBG)
            def _():
                with_weights(project_out, g)

            is_ring = ring.astype(I32)
            return t + is_ring, r + 1 - is_ring

        lax.fori_loop(0, NP, second, (jnp.int32(0), jnp.int32(0)))
        x3 = x2 + jnp.sum(ys[...], axis=0, keepdims=True)
        with_weights(ffn, x3)
        o_ref[...] = (x3 + fo[...])[0:1, :].astype(o_ref.dtype)

    return kernel


@jax.jit
def pallas_interleave_layers__gqa_block_cached__dense_activation_mish__decode_kernel(
    A_x: jax.Array,
    A_k_cache: jax.Array,
    A_v_cache: jax.Array,
    A_wq: jax.Array,
    A_wo: jax.Array,
    B_x: jax.Array,
    B_w1: jax.Array,
    B_b1: jax.Array,
    B_w2: jax.Array,
):
    del B_x
    hbm = pl.BlockSpec(memory_space=pl.ANY)
    vmem = pl.BlockSpec(memory_space=pltpu.VMEM)
    out = pl.pallas_call(
        _make_kernel(),
        out_shape=jax.ShapeDtypeStruct((1, D), A_x.dtype),
        in_specs=[vmem, vmem] + [hbm] * 6,
        out_specs=vmem,
        scratch_shapes=[
            pltpu.VMEM((END, DH), I32),
            pltpu.VMEM((HKV, 8, DH), BF),
            pltpu.VMEM((HKV, 8, DH), F32),
            pltpu.VMEM((HKV, 8, DH), F32),
            pltpu.VMEM((HKV, 8, DH), F32),
            pltpu.VMEM((8, D), F32),
            pltpu.VMEM((8, D), F32),
        ] + [pltpu.SMEM((NP,), I32)] * 6 + [
            pltpu.SMEM((HKV,), I32),
            pltpu.SMEM((16,), I32),
            pltpu.SMEM((1,), I32),
            pltpu.SemaphoreType.DMA((S,)),
            pltpu.SemaphoreType.DMA((4,)),
        ],
        compiler_params=pltpu.CompilerParams(vmem_limit_bytes=128 * 1024 * 1024, disable_bounds_checks=True),
    )(A_x.reshape(1, D), B_b1.reshape(F // DH, DH), A_k_cache.reshape(HKV * SK, DH),
      A_v_cache.reshape(HKV * SK, DH), A_wq, A_wo, B_w1, B_w2)
    return out.reshape(1, 1, D)
```
